```python
import jax
import jax.numpy as jnp

def _softmax(x, axis=-1):
    return jax.nn.softmax(x, axis=axis)

def _gelu(x):
    return jax.nn.gelu(x, approximate=True)

def _silu(x):
    return jax.nn.silu(x)

def _sigmoid(x):
    return jax.nn.sigmoid(x)

def _layernorm(x, axis=-1, eps=1e-05):
    m = jnp.mean(x, axis=axis, keepdims=True)
    v = jnp.var(x, axis=axis, keepdims=True)
    return (x - m) / jnp.sqrt(v + eps)

def _scatter_add(tgt, idx, src, axis=0):
    return tgt.at[idx].add(src)

def _segment_sum(src, seg, n):
    return jax.ops.segment_sum(src, seg, n)

class _Rng:

    def __init__(self, key):
        self._k = key

    def _next(self):
        self._k, sub = jax.random.split(self._k)
        return sub

    def normal(self, shape):
        return jax.random.normal(self._next(), shape, dtype=jnp.bfloat16)

    def randint(self, lo, hi, shape):
        return jax.random.randint(self._next(), shape, lo, hi, dtype=jnp.int32)

    def uniform(self, shape, lo=0.0, hi=1.0):
        return jax.random.uniform(self._next(), shape, jnp.bfloat16, lo, hi)

    def permutation(self, n):
        return jax.random.permutation(self._next(), n)
kernel_name = 'adaLN_cond__sliding_block_cached__dense_activation_gelu__decode'

def setup_inputs():
    _rng = _Rng(jax.random.key(int.from_bytes(__import__("os").urandom(4), "little")))
    _w = lambda a: (lambda t: t.astype(jnp.bfloat16) if jnp.issubdtype(t.dtype, jnp.floating) else t)(jnp.asarray(a))

    def _A_setup():
        B, Sq, D = (4, 1, 640)
        Hq, Hkv, Sk, Dh = (32, 32, 8192, 128)
        assert Hq % Hkv == 0, (Hq, Hkv)
        return {'x': _w((lambda *s: _rng.normal(s) * 0.05)(B, Sq, D)), 'k_cache': _w((lambda *s: _rng.normal(s) * 0.05)(B, Hkv, Sk, Dh)), 'v_cache': _w((lambda *s: _rng.normal(s) * 0.05)(B, Hkv, Sk, Dh)), 'wq': _w((lambda *s: _rng.normal(s) * 0.05)(D, Hq * Dh) * D ** (-0.5)), 'wo': _w((lambda *s: _rng.normal(s) * 0.05)(Hq * Dh, D) * (Hq * Dh) ** (-0.5))}
    _A_in = _A_setup()

    def _B_setup():
        B, S, D, F = (4, 1, 640, 1728)
        return {'x': _w((lambda *s: _rng.normal(s) * 0.05)(B, S, D)), 'w1': _w((lambda *s: _rng.normal(s) * 0.05)(D, F) * D ** (-0.5)), 'b1': _w((lambda *s: _rng.normal(s) * 0.05)(F) * 0.01), 'w2': _w((lambda *s: _rng.normal(s) * 0.05)(F, D) * F ** (-0.5)), 'b2': _w((lambda *s: _rng.normal(s) * 0.05)(D) * 0.01)}
    _B_in = _B_setup()
    return {'A_x': _A_in['x'], 'A_k_cache': _A_in['k_cache'], 'A_v_cache': _A_in['v_cache'], 'A_wq': _A_in['wq'], 'A_wo': _A_in['wo'], 'B_x': _B_in['x'], 'B_w1': _B_in['w1'], 'B_b1': _B_in['b1'], 'B_w2': _B_in['w2'], 'B_b2': _B_in['b2'], 'c': _w((lambda *s: _rng.normal(s) * 0.05)(4, 640)), 'w_mod': _w((lambda *s: _rng.normal(s) * 0.05)(640, 6 * 640) * 640 ** (-0.5))}

def reference(A_x, A_k_cache, A_v_cache, A_wq, A_wo, B_x, B_w1, B_b1, B_w2, B_b2, c, w_mod):

    def _A_ref(x, k_cache, v_cache, wq, wo):
        B, Sq, D = x.shape
        Hq, Dh = (32, 128)
        Hkv, Sk = (k_cache.shape[1], k_cache.shape[2])
        W = min(4096, max(256, Sk // 4))
        rep = Hq // Hkv
        q = (lambda x, *d: x.transpose(*d))((x @ wq).reshape(B, Sq, Hq, Dh), 0, 2, 1, 3)
        k = jnp.repeat(k_cache[:, :, Sk - W:, :], rep, axis=1)
        v = jnp.repeat(v_cache[:, :, Sk - W:, :], rep, axis=1)
        scores = jnp.einsum('bhqd,bhkd->bhqk', q, k) * Dh ** (-0.5)
        p = _softmax(scores, axis=-1)
        o = jnp.einsum('bhqk,bhkd->bhqd', p, v)
        return (lambda x, *d: x.transpose(*d))(o, 0, 2, 1, 3).reshape(B, Sq, Hq * Dh) @ wo

    def _B_ref(x, w1, b1, w2, b2):
        h = jnp.einsum('bsd,df->bsf', x, w1) + b1
        h = _gelu(h)
        return jnp.einsum('bsf,fd->bsd', h, w2) + b2
    x = A_x
    mod = (_silu(c) @ w_mod).reshape(c.shape[0], 6, 1, -1)
    sa, ca, ga, sb, cb, gb = (mod[:, 0].copy(), mod[:, 1].copy(), mod[:, 2].copy(), mod[:, 3].copy(), mod[:, 4].copy(), mod[:, 5].copy())
    h = _layernorm(x, axis=-1) * (1 + ca) + sa
    x = x + ga * _A_ref(h, A_k_cache, A_v_cache, A_wq, A_wo)
    h = _layernorm(x, axis=-1) * (1 + cb) + sb
    x = x + gb * _B_ref(h, B_w1, B_b1, B_w2, B_b2)
    return x
```

```python
import functools

import jax
import jax.numpy as jnp
import jax.experimental.pallas as pl
import jax.experimental.pallas.tpu as pltpu

HQ, DH = 32, 128
ROWS = 8
F32, BF16 = jnp.float32, jnp.bfloat16
_NT = (((1,), (1,)), ((), ()))


def _layernorm(x):
    m = jnp.mean(x, axis=-1, keepdims=True)
    d = x - m
    v = jnp.mean(d * d, axis=-1, keepdims=True)
    return d / jnp.sqrt(v + 1e-5)


def _pad_rows(x):
    return jnp.concatenate([x, jnp.zeros((ROWS - x.shape[0], x.shape[1]), x.dtype)], axis=0)


def _kernel(x_hbm, k_hbm, v_hbm, wq_hbm, wo_hbm, w1t_hbm, b1_hbm, w2_hbm, b2_hbm, c_hbm, wmod_hbm,
            out_ref,
            x_v, c_v, b1_v, b2_v, wmod_v, wq_v, wo_v, w1t_v, w2_v, k_v, v_v, q_v, o_v,
            kv_sem, w_sem, *, nslots, window, w2_splits):
    nb, d = x_v.shape
    sk = k_hbm.shape[2]

    def kv_copy(which, h, slot):
        src, dst = (k_hbm, k_v) if which == 0 else (v_hbm, v_v)
        return pltpu.make_async_copy(
            src.at[:, h, pl.ds(sk - window, window), :], dst.at[slot], kv_sem.at[which, slot])

    def start_kv(h, slot):
        kv_copy(0, h, slot).start(priority=0)
        kv_copy(1, h, slot).start(priority=1)

    cp = lambda i, s, t: pltpu.make_async_copy(s, t, w_sem.at[i])
    c_wmod, c_wq = cp(0, wmod_hbm, wmod_v), cp(1, wq_hbm, wq_v)
    small = [cp(2, c_hbm, c_v), cp(3, x_hbm, x_v), cp(4, b1_hbm, b1_v), cp(5, b2_hbm, b2_v)]
    c_wo, c_w1 = cp(6, wo_hbm, wo_v), cp(7, w1t_hbm, w1t_v)
    c_w2 = [cp(8 + i, w2_hbm.at[pl.ds(a, b - a)], w2_v.at[pl.ds(a, b - a)])
            for i, (a, b) in enumerate(zip(w2_splits[:-1], w2_splits[1:]))]

    c_wmod.start(priority=0)
    c_wq.start(priority=1)
    for s in small:
        s.start(priority=0)
    for h in range(nslots):
        start_kv(h, h)

    for s in small:
        s.wait()
    c_wmod.wait()
    cf = _pad_rows(c_v[...].astype(F32))
    mod = jnp.dot((cf * jax.nn.sigmoid(cf)).astype(BF16), wmod_v[...], preferred_element_type=F32)
    sa, ca, ga, sb, cb, gb = (mod[:, i * d:(i + 1) * d] for i in range(6))
    x = _pad_rows(x_v[...].astype(F32))
    h1 = _layernorm(x) * (1.0 + ca) + sa
    c_wq.wait()
    q = jnp.dot(h1.astype(BF16), wq_v[...], preferred_element_type=F32)
    for h in range(HQ):
        q_v[h] = q[:, h * DH:(h + 1) * DH]

    def head(h, _):
        slot = h % nslots
        qh = q_v[h].astype(BF16)
        kv_copy(0, h, slot).wait()
        row = jax.lax.broadcasted_iota(jnp.int32, (ROWS, window), 0)
        s = None
        for b in range(nb):
            sb_ = jax.lax.dot_general(qh, k_v[slot, b], _NT, preferred_element_type=F32)
            s = sb_ if s is None else jnp.where(row == b, sb_, s)
        s = s * (DH ** -0.5)
        p = jnp.exp(s - jnp.max(s, axis=-1, keepdims=True))
        l = jnp.sum(p, axis=-1, keepdims=True)
        pb = p.astype(BF16)
        kv_copy(1, h, slot).wait()
        row = jax.lax.broadcasted_iota(jnp.int32, (ROWS, DH), 0)
        o = None
        for b in range(nb):
            ob = jnp.dot(pb, v_v[slot, b], preferred_element_type=F32)
            o = ob if o is None else jnp.where(row == b, ob, o)
        o_v[h] = o / l

        @pl.when(h + nslots < HQ)
        def _():
            start_kv(h + nslots, slot)

        @pl.when(h + nslots == HQ)
        def _():
            c_wo.start(priority=0)
            c_w1.start(priority=1)
            for i, c_ in enumerate(c_w2):
                c_.start(priority=1)

    jax.lax.fori_loop(0, HQ, head, None)

    o = jnp.concatenate([o_v[h] for h in range(HQ)], axis=1).astype(BF16)
    c_wo.wait()
    x = x + ga * jnp.dot(o, wo_v[...], preferred_element_type=F32)
    h2 = _layernorm(x) * (1.0 + cb) + sb
    c_w1.wait()
    u = jax.lax.dot_general(h2.astype(BF16), w1t_v[...], _NT, preferred_element_type=F32)
    u = u + b1_v[...].astype(F32)[None, :]
    g = jax.nn.gelu(u, approximate=True).astype(BF16)
    y = jnp.broadcast_to(b2_v[...].astype(F32)[None, :], (ROWS, d))
    for c_, a, b in zip(c_w2, w2_splits[:-1], w2_splits[1:]):
        c_.wait()
        y = y + jnp.dot(g[:, a:b], w2_v[a:b, :], preferred_element_type=F32)
    out_ref[...] = (x + gb * y)[:nb].astype(out_ref.dtype)


def _build(nslots=3, w2_splits=(0, 1280, 1728)):
    def fn(A_x, A_k_cache, A_v_cache, A_wq, A_wo, B_x, B_w1, B_b1, B_w2, B_b2, c, w_mod):
        del B_x
        nb, _, d = A_x.shape
        sk = A_k_cache.shape[2]
        window = min(4096, max(256, sk // 4))
        f = B_w1.shape[1]
        dt = A_x.dtype
        ins = (A_x.reshape(nb, d), A_k_cache, A_v_cache, A_wq, A_wo, B_w1.T, B_b1, B_w2, B_b2, c, w_mod)
        out = pl.pallas_call(
            functools.partial(_kernel, nslots=nslots, window=window, w2_splits=w2_splits),
            out_shape=jax.ShapeDtypeStruct((nb, d), dt),
            in_specs=[pl.BlockSpec(memory_space=pltpu.HBM)] * len(ins),
            out_specs=pl.BlockSpec(memory_space=pltpu.VMEM),
            scratch_shapes=[
                pltpu.VMEM((nb, d), dt), pltpu.VMEM((nb, d), dt),
                pltpu.VMEM((f,), dt), pltpu.VMEM((d,), dt),
                pltpu.VMEM(w_mod.shape, dt), pltpu.VMEM(A_wq.shape, dt), pltpu.VMEM(A_wo.shape, dt),
                pltpu.VMEM((f, d), dt), pltpu.VMEM((f, d), dt),
                pltpu.VMEM((nslots, nb, window, DH), dt), pltpu.VMEM((nslots, nb, window, DH), dt),
                pltpu.VMEM((HQ, ROWS, DH), F32), pltpu.VMEM((HQ, ROWS, DH), F32),
                pltpu.SemaphoreType.DMA((2, nslots)),
                pltpu.SemaphoreType.DMA((8 + len(w2_splits) - 1,)),
            ],
            compiler_params=pltpu.CompilerParams(vmem_limit_bytes=100 * 2**20),
        )(*ins)
        return out.reshape(A_x.shape)
    return fn


@jax.jit
def pallas_adaLN_cond__sliding_block_cached__dense_activation_gelu__decode_kernel(
    A_x, A_k_cache, A_v_cache, A_wq, A_wo, B_x, B_w1, B_b1, B_w2, B_b2, c, w_mod,
):
    return _build()(A_x, A_k_cache, A_v_cache, A_wq, A_wo, B_x, B_w1, B_b1, B_w2, B_b2, c, w_mod)
```

```python
import functools

import jax
import jax.numpy as jnp
import jax.experimental.pallas as pl
import jax.experimental.pallas.tpu as pltpu

HQ, DH = 32, 128
ROWS = 8
F32, BF16 = jnp.float32, jnp.bfloat16
_NT = (((1,), (1,)), ((), ()))


def _layernorm(x):
    m = jnp.mean(x, axis=-1, keepdims=True)
    d = x - m
    v = jnp.mean(d * d, axis=-1, keepdims=True)
    return d / jnp.sqrt(v + 1e-5)


def _pad_rows(x):
    return jnp.concatenate([x, jnp.zeros((ROWS - x.shape[0], x.shape[1]), x.dtype)], axis=0)


def _kernel(x_hbm, k_hbm, v_hbm, wq_hbm, wo_hbm, w1t_hbm, b1_hbm, w2_hbm, b2_hbm, c_hbm, wmod_hbm,
            out_ref,
            x_v, c_v, b1_v, b2_v, wmod_v, wq_v, wo_v, w1t_v, w2_v, k_v, v_v, q_v, o_v,
            side_s, kv_sem, w_sem, side_sem, *, nslots, window, w2_splits, side):
    nb, d = x_v.shape
    sk = k_hbm.shape[2]

    def kv_copy(which, h, slot):
        src, dst, n = (k_hbm, k_v, window - side) if which == 0 else (v_hbm, v_v, window)
        return pltpu.make_async_copy(
            src.at[:, h, pl.ds(sk - window, n), :], dst.at[slot, :, pl.ds(0, n), :],
            kv_sem.at[which, slot])

    def side_in(h):
        return pltpu.make_async_copy(
            k_hbm.at[:, h, pl.ds(sk - side, side), :], side_s.at[h % 2], side_sem.at[0, h % 2])

    def side_out(h):
        return pltpu.make_async_copy(
            side_s.at[h % 2], k_v.at[h % nslots, :, pl.ds(window - side, side), :],
            side_sem.at[1, h % 2])

    def start_kv(h, slot):
        kv_copy(0, h, slot).start(priority=0)
        kv_copy(1, h, slot).start(priority=1)

    cp = lambda i, s, t: pltpu.make_async_copy(s, t, w_sem.at[i])
    c_wmod, c_wq = cp(0, wmod_hbm, wmod_v), cp(1, wq_hbm, wq_v)
    small = [cp(2, c_hbm, c_v), cp(3, x_hbm, x_v), cp(4, b1_hbm, b1_v), cp(5, b2_hbm, b2_v)]
    c_wo, c_w1 = cp(6, wo_hbm, wo_v), cp(7, w1t_hbm, w1t_v)
    c_w2 = [cp(8 + i, w2_hbm.at[pl.ds(a, b - a)], w2_v.at[pl.ds(a, b - a)])
            for i, (a, b) in enumerate(zip(w2_splits[:-1], w2_splits[1:]))]

    c_wmod.start(priority=0)
    c_wq.start(priority=1)
    for s in small:
        s.start(priority=0)
    side_in(0).start()
    side_in(1).start()
    for h in range(nslots):
        start_kv(h, h)

    for s in small:
        s.wait()
    c_wmod.wait()
    side_in(0).wait()
    side_out(0).start()
    cf = _pad_rows(c_v[...].astype(F32))
    mod = jnp.dot((cf * jax.nn.sigmoid(cf)).astype(BF16), wmod_v[...], preferred_element_type=F32)
    sa, ca, ga, sb, cb, gb = (mod[:, i * d:(i + 1) * d] for i in range(6))
    x = _pad_rows(x_v[...].astype(F32))
    h1 = _layernorm(x) * (1.0 + ca) + sa
    c_wq.wait()
    q = jnp.dot(h1.astype(BF16), wq_v[...], preferred_element_type=F32)
    for h in range(HQ):
        q_v[h] = q[:, h * DH:(h + 1) * DH]

    def head(h, _):
        slot = h % nslots
        qh = q_v[h].astype(BF16)
        side_out(h).wait()

        @pl.when(h + 1 < HQ)
        def _():
            side_in(h + 1).wait()
            side_out(h + 1).start()

        @pl.when(h + 2 < HQ)
        def _():
            side_in(h + 2).start()

        kv_copy(0, h, slot).wait()
        row = jax.lax.broadcasted_iota(jnp.int32, (ROWS, window), 0)
        s = None
        for b in range(nb):
            sb_ = jax.lax.dot_general(qh, k_v[slot, b], _NT, preferred_element_type=F32)
            s = sb_ if s is None else jnp.where(row == b, sb_, s)
        s = s * (DH ** -0.5)
        p = jnp.exp(s - jnp.max(s, axis=-1, keepdims=True))
        l = jnp.sum(p, axis=-1, keepdims=True)
        pb = p.astype(BF16)
        kv_copy(1, h, slot).wait()
        row = jax.lax.broadcasted_iota(jnp.int32, (ROWS, DH), 0)
        o = None
        for b in range(nb):
            ob = jnp.dot(pb, v_v[slot, b], preferred_element_type=F32)
            o = ob if o is None else jnp.where(row == b, ob, o)
        o_v[h] = o / l

        @pl.when(h + nslots < HQ)
        def _():
            start_kv(h + nslots, slot)

        @pl.when(h + nslots == HQ)
        def _():
            c_wo.start(priority=0)
            c_w1.start(priority=1)
            for i, c_ in enumerate(c_w2):
                c_.start(priority=1)

    jax.lax.fori_loop(0, HQ, head, None)

    o = jnp.concatenate([o_v[h] for h in range(HQ)], axis=1).astype(BF16)
    c_wo.wait()
    x = x + ga * jnp.dot(o, wo_v[...], preferred_element_type=F32)
    h2 = _layernorm(x) * (1.0 + cb) + sb
    c_w1.wait()
    u = jax.lax.dot_general(h2.astype(BF16), w1t_v[...], _NT, preferred_element_type=F32)
    u = u + b1_v[...].astype(F32)[None, :]
    g = jax.nn.gelu(u, approximate=True).astype(BF16)
    y = jnp.broadcast_to(b2_v[...].astype(F32)[None, :], (ROWS, d))
    for c_, a, b in zip(c_w2, w2_splits[:-1], w2_splits[1:]):
        c_.wait()
        y = y + jnp.dot(g[:, a:b], w2_v[a:b, :], preferred_element_type=F32)
    out_ref[...] = (x + gb * y)[:nb].astype(out_ref.dtype)


def _build(nslots=3, w2_splits=(0, 1280, 1728), side=96, cp=()):
    def fn(A_x, A_k_cache, A_v_cache, A_wq, A_wo, B_x, B_w1, B_b1, B_w2, B_b2, c, w_mod):
        del B_x
        nb, _, d = A_x.shape
        sk = A_k_cache.shape[2]
        window = min(4096, max(256, sk // 4))
        f = B_w1.shape[1]
        dt = A_x.dtype
        ins = (A_x.reshape(nb, d), A_k_cache, A_v_cache, A_wq, A_wo, B_w1.T, B_b1, B_w2, B_b2, c, w_mod)
        out = pl.pallas_call(
            functools.partial(_kernel, nslots=nslots, window=window, w2_splits=w2_splits, side=side),
            out_shape=jax.ShapeDtypeStruct((nb, d), dt),
            in_specs=[pl.BlockSpec(memory_space=pltpu.HBM)] * len(ins),
            out_specs=pl.BlockSpec(memory_space=pltpu.VMEM),
            scratch_shapes=[
                pltpu.VMEM((nb, d), dt), pltpu.VMEM((nb, d), dt),
                pltpu.VMEM((f,), dt), pltpu.VMEM((d,), dt),
                pltpu.VMEM(w_mod.shape, dt), pltpu.VMEM(A_wq.shape, dt), pltpu.VMEM(A_wo.shape, dt),
                pltpu.VMEM((f, d), dt), pltpu.VMEM((f, d), dt),
                pltpu.VMEM((nslots, nb, window, DH), dt), pltpu.VMEM((nslots, nb, window, DH), dt),
                pltpu.VMEM((HQ, ROWS, DH), F32), pltpu.VMEM((HQ, ROWS, DH), F32),
                pltpu.SMEM((2, nb, side, DH), dt),
                pltpu.SemaphoreType.DMA((2, nslots)),
                pltpu.SemaphoreType.DMA((8 + len(w2_splits) - 1,)),
                pltpu.SemaphoreType.DMA((2, 2)),
            ],
            compiler_params=pltpu.CompilerParams(vmem_limit_bytes=100 * 2**20, **dict(cp)),
        )(*ins)
        return out.reshape(A_x.shape)
    return fn


@jax.jit
def pallas_adaLN_cond__sliding_block_cached__dense_activation_gelu__decode_kernel(
    A_x, A_k_cache, A_v_cache, A_wq, A_wo, B_x, B_w1, B_b1, B_w2, B_b2, c, w_mod,
):
    return _build()(A_x, A_k_cache, A_v_cache, A_wq, A_wo, B_x, B_w1, B_b1, B_w2, B_b2, c, w_mod)
```

```python
import functools

import jax
import jax.numpy as jnp
import jax.experimental.pallas as pl
import jax.experimental.pallas.tpu as pltpu

HQ, DH = 32, 128
ROWS = 8
F32, BF16 = jnp.float32, jnp.bfloat16
_NT = (((1,), (1,)), ((), ()))
SIDE_Q, MAIN_Q = 0, 1


def _layernorm(x):
    m = jnp.mean(x, axis=-1, keepdims=True)
    d = x - m
    v = jnp.mean(d * d, axis=-1, keepdims=True)
    return d / jnp.sqrt(v + 1e-5)


def _pad_rows(x):
    return jnp.concatenate([x, jnp.zeros((ROWS - x.shape[0], x.shape[1]), x.dtype)], axis=0)


def _kernel(x_hbm, k_hbm, v_hbm, wq_hbm, wo_hbm, w1t_hbm, b1_hbm, w2_hbm, b2_hbm, c_hbm, wmod_hbm,
            out_ref,
            x_v, c_v, b1_v, b2_v, wmod_v, wq_v, wo_v, w1t_v, w2_v, k_v, v_v, q_v, o_v,
            kside_s, wside_s, kv_sem, w_sem, side_sem, *, w2_splits, k_queue):
    nb, d = x_v.shape
    f = w1t_v.shape[0]
    sk = k_hbm.shape[2]
    nslots, _, window, _ = k_v.shape
    kside, wside = kside_s.shape[2], wside_s.shape[1]
    copy = pltpu.make_async_copy

    def k_copy(h):
        n = window - kside
        return copy(k_hbm.at[:, h, pl.ds(sk - window, n), :],
                    k_v.at[h % nslots, :, pl.ds(0, n), :], kv_sem.at[0, h % nslots])

    def v_copy(h):
        return copy(v_hbm.at[:, h, pl.ds(sk - window, window), :],
                    v_v.at[h % nslots], kv_sem.at[1, h % nslots])

    def kside_in(h):
        return copy(k_hbm.at[:, h, pl.ds(sk - kside, kside), :],
                    kside_s.at[h % 2], side_sem.at[0, h % 2])

    def kside_out(h):
        return copy(kside_s.at[h % 2],
                    k_v.at[h % nslots, :, pl.ds(window - kside, kside), :], side_sem.at[1, h % 2])

    def start_kv(h):
        k_copy(h).start(priority=k_queue)
        v_copy(h).start(priority=MAIN_Q)

    def rows(src, dst, a, b, i):
        return copy(src.at[pl.ds(a, b - a)], dst.at[pl.ds(a, b - a)], w_sem.at[i])

    wmod_copy = copy(wmod_hbm, wmod_v, w_sem.at[0])
    wq_copy = copy(wq_hbm, wq_v, w_sem.at[1])
    wo_copy = copy(wo_hbm, wo_v, w_sem.at[2])
    small = [copy(s, t, w_sem.at[3 + i]) for i, (s, t) in enumerate(
        ((c_hbm, c_v), (x_hbm, x_v), (b1_hbm, b1_v), (b2_hbm, b2_v)))]
    w1_copy = rows(w1t_hbm, w1t_v, wside, f, 7)
    w2_copies = [rows(w2_hbm, w2_v, a, b, 8 + i) for i, (a, b) in enumerate(
        zip((wside,) + w2_splits[1:-1], w2_splits[1:]))]
    wside_in = [copy(w.at[pl.ds(0, wside)], wside_s.at[i], side_sem.at[2, i])
                for i, w in enumerate((w1t_hbm, w2_hbm))]
    wside_out = [copy(wside_s.at[i], w.at[pl.ds(0, wside)], side_sem.at[3, i])
                 for i, w in enumerate((w1t_v, w2_v))]

    wmod_copy.start(priority=MAIN_Q)
    for c_ in small:
        c_.start(priority=SIDE_Q)
    wq_copy.start(priority=MAIN_Q)
    kside_in(0).start(priority=SIDE_Q)
    kside_in(1).start(priority=SIDE_Q)
    for h in range(nslots):
        start_kv(h)

    for c_ in small:
        c_.wait()
    wmod_copy.wait()
    kside_in(0).wait()
    kside_out(0).start(priority=SIDE_Q)
    cf = _pad_rows(c_v[...].astype(F32))
    mod = jnp.dot((cf * jax.nn.sigmoid(cf)).astype(BF16), wmod_v[...], preferred_element_type=F32)
    sa, ca, ga, sb, cb, gb = (mod[:, i * d:(i + 1) * d] for i in range(6))
    x = _pad_rows(x_v[...].astype(F32))
    h1 = _layernorm(x) * (1.0 + ca) + sa
    wq_copy.wait()
    q = jnp.dot(h1.astype(BF16), wq_v[...], preferred_element_type=F32)
    for h in range(HQ):
        q_v[h] = q[:, h * DH:(h + 1) * DH]

    def head(h, _):
        slot = h % nslots
        kside_out(h).wait()

        @pl.when(h + 1 < HQ)
        def _():
            kside_in(h + 1).wait()
            kside_out(h + 1).start(priority=SIDE_Q)

        @pl.when(h + 2 < HQ)
        def _():
            kside_in(h + 2).start(priority=SIDE_Q)

        @pl.when(h + 2 == HQ)
        def _():
            wside_in[0].start(priority=SIDE_Q)

        @pl.when(h + 1 == HQ)
        def _():
            wside_in[0].wait()
            wside_out[0].start(priority=SIDE_Q)
            wside_in[1].start(priority=SIDE_Q)

        qh = q_v[h].astype(BF16)
        k_copy(h).wait()
        row = jax.lax.broadcasted_iota(jnp.int32, (ROWS, window), 0)
        s = None
        for b in range(nb):
            s_b = jax.lax.dot_general(qh, k_v[slot, b], _NT, preferred_element_type=F32)
            s = s_b if s is None else jnp.where(row == b, s_b, s)
        s = s * (DH ** -0.5)
        p = jnp.exp(s - jnp.max(s, axis=-1, keepdims=True))
        l = jnp.sum(p, axis=-1, keepdims=True)
        pb = p.astype(BF16)
        v_copy(h).wait()
        row = jax.lax.broadcasted_iota(jnp.int32, (ROWS, DH), 0)
        o = None
        for b in range(nb):
            o_b = jnp.dot(pb, v_v[slot, b], preferred_element_type=F32)
            o = o_b if o is None else jnp.where(row == b, o_b, o)
        o_v[h] = o / l

        @pl.when(h + nslots < HQ)
        def _():
            start_kv(h + nslots)

        @pl.when(h + nslots == HQ)
        def _():
            for c_ in [wo_copy, w1_copy] + w2_copies:
                c_.start(priority=MAIN_Q)

    jax.lax.fori_loop(0, HQ, head, None)

    wside_in[1].wait()
    wside_out[1].start(priority=SIDE_Q)
    o = jnp.concatenate([o_v[h] for h in range(HQ)], axis=1).astype(BF16)
    wo_copy.wait()
    x = x + ga * jnp.dot(o, wo_v[...], preferred_element_type=F32)
    h2 = _layernorm(x) * (1.0 + cb) + sb
    wside_out[0].wait()
    w1_copy.wait()
    u = jax.lax.dot_general(h2.astype(BF16), w1t_v[...], _NT, preferred_element_type=F32)
    u = u + b1_v[...].astype(F32)[None, :]
    g = jax.nn.gelu(u, approximate=True).astype(BF16)
    y = jnp.broadcast_to(b2_v[...].astype(F32)[None, :], (ROWS, d))
    wside_out[1].wait()
    for c_, a, b in zip(w2_copies, w2_splits[:-1], w2_splits[1:]):
        c_.wait()
        y = y + jnp.dot(g[:, a:b], w2_v[a:b, :], preferred_element_type=F32)
    out_ref[...] = (x + gb * y)[:nb].astype(out_ref.dtype)


def _build(nslots=2, kside=96, wside=128, w2_cuts=(1280,), k_queue=SIDE_Q):
    def fn(A_x, A_k_cache, A_v_cache, A_wq, A_wo, B_x, B_w1, B_b1, B_w2, B_b2, c, w_mod):
        del B_x
        nb, _, d = A_x.shape
        sk = A_k_cache.shape[2]
        window = min(4096, max(256, sk // 4))
        f = B_w1.shape[1]
        dt = A_x.dtype
        w2_splits = (0, *w2_cuts, f)
        ins = (A_x.reshape(nb, d), A_k_cache, A_v_cache, A_wq, A_wo, B_w1.T, B_b1, B_w2, B_b2, c, w_mod)
        out = pl.pallas_call(
            functools.partial(_kernel, w2_splits=w2_splits, k_queue=k_queue),
            out_shape=jax.ShapeDtypeStruct((nb, d), dt),
            in_specs=[pl.BlockSpec(memory_space=pltpu.HBM)] * len(ins),
            out_specs=pl.BlockSpec(memory_space=pltpu.VMEM),
            scratch_shapes=[
                pltpu.VMEM((nb, d), dt), pltpu.VMEM((nb, d), dt),
                pltpu.VMEM((f,), dt), pltpu.VMEM((d,), dt),
                pltpu.VMEM(w_mod.shape, dt), pltpu.VMEM(A_wq.shape, dt), pltpu.VMEM(A_wo.shape, dt),
                pltpu.VMEM((f, d), dt), pltpu.VMEM((f, d), dt),
                pltpu.VMEM((nslots, nb, window, DH), dt), pltpu.VMEM((nslots, nb, window, DH), dt),
                pltpu.VMEM((HQ, ROWS, DH), F32), pltpu.VMEM((HQ, ROWS, DH), F32),
                pltpu.SMEM((2, nb, kside, DH), dt), pltpu.SMEM((2, wside, d), dt),
                pltpu.SemaphoreType.DMA((2, nslots)),
                pltpu.SemaphoreType.DMA((7 + len(w2_splits),)),
                pltpu.SemaphoreType.DMA((4, 2)),
            ],
            compiler_params=pltpu.CompilerParams(vmem_limit_bytes=100 * 2**20),
        )(*ins)
        return out.reshape(A_x.shape)
    return fn


@jax.jit
def pallas_adaLN_cond__sliding_block_cached__dense_activation_gelu__decode_kernel(
    A_x, A_k_cache, A_v_cache, A_wq, A_wo, B_x, B_w1, B_b1, B_w2, B_b2, c, w_mod,
):
    return _build()(A_x, A_k_cache, A_v_cache, A_wq, A_wo, B_x, B_w1, B_b1, B_w2, B_b2, c, w_mod)
```
